```python
import os as _os
_os.environ.setdefault('JAX_PLATFORMS', 'cpu')
import jax
import jax.numpy as jnp

def _softmax(x, axis=-1):
    return jax.nn.softmax(x, axis=axis)

def _gelu(x):
    return jax.nn.gelu(x, approximate=True)

def _silu(x):
    return jax.nn.silu(x)

def _sigmoid(x):
    return jax.nn.sigmoid(x)

def _layernorm(x, axis=-1, eps=1e-05):
    m = jnp.mean(x, axis=axis, keepdims=True)
    v = jnp.var(x, axis=axis, keepdims=True)
    return (x - m) / jnp.sqrt(v + eps)

def _scatter_add(tgt, idx, src, axis=0):
    return tgt.at[idx].add(src)

def _segment_sum(src, seg, n):
    return jax.ops.segment_sum(src, seg, n)

class _Rng:

    def __init__(self, key):
        self._k = key

    def _next(self):
        self._k, sub = jax.random.split(self._k)
        return sub

    def normal(self, shape):
        return jax.random.normal(self._next(), shape, dtype=jnp.bfloat16)

    def randint(self, lo, hi, shape):
        return jax.random.randint(self._next(), shape, lo, hi, dtype=jnp.int32)

    def uniform(self, shape, lo=0.0, hi=1.0):
        return jax.random.uniform(self._next(), shape, jnp.bfloat16, lo, hi)

    def permutation(self, n):
        return jax.random.permutation(self._next(), n)
kernel_name = 'parallel_sum__memory_aug_recurrent_mem_tr__dense_activation_silu__prompt'

def setup_inputs():
    _rng = _Rng(jax.random.key(int.from_bytes(__import__("os").urandom(4), "little")))
    _w = lambda a: (lambda t: t.astype(jnp.bfloat16) if jnp.issubdtype(t.dtype, jnp.floating) else t)(jnp.asarray(a))

    def _A_setup():
        B, S, Dm = (1, 2048, 448)
        H, Dh = (16, 256)
        M, seg = (8, 32)
        seg = min(seg, S)
        S = S // seg * seg
        return {'x': _w((lambda *s: _rng.normal(s) * 0.05)(B, S, Dm)), 'mem0': _w((lambda *s: _rng.normal(s) * 0.2)(B, M, Dm)), 'Wq': _w((lambda *s: _rng.normal(s) * 0.8)(Dm, H, Dh) * Dm ** (-0.5)), 'Wk': _w((lambda *s: _rng.normal(s) * 0.8)(Dm, H, Dh) * Dm ** (-0.5)), 'Wv': _w((lambda *s: _rng.normal(s) * 0.2)(Dm, H, Dh) * Dm ** (-0.5)), 'Wo': _w((lambda *s: _rng.normal(s) * 0.2)(H, Dh, Dm) * (H * Dh) ** (-0.5)), 'seg_len': seg}
    _A_in = _A_setup()

    def _B_setup():
        B, S, D, F = (1, 2048, 448, 1792)
        return {'x': _w((lambda *s: _rng.normal(s) * 0.05)(B, S, D)), 'w1': _w((lambda *s: _rng.normal(s) * 0.05)(D, F) * D ** (-0.5)), 'w2': _w((lambda *s: _rng.normal(s) * 0.05)(F, D) * F ** (-0.5))}
    _B_in = _B_setup()
    return {'A_x': _A_in['x'], 'A_mem0': _A_in['mem0'], 'A_Wq': _A_in['Wq'], 'A_Wk': _A_in['Wk'], 'A_Wv': _A_in['Wv'], 'A_Wo': _A_in['Wo'], 'A_seg_len': _A_in['seg_len'], 'B_x': _B_in['x'], 'B_w1': _B_in['w1'], 'B_w2': _B_in['w2']}

def reference(A_x, A_mem0, A_Wq, A_Wk, A_Wv, A_Wo, A_seg_len, B_x, B_w1, B_w2):

    def _A_ref(x, mem0, Wq, Wk, Wv, Wo, seg_len):
        B, S, Dm = x.shape
        H, Dh = (Wq.shape[1], Wq.shape[2])
        M = mem0.shape[1]
        scale = Dh ** (-0.5)
        n_seg = S // seg_len
        L = M + seg_len
        idx = jnp.arange(L)
        mask = (idx[:, None] < M) | (idx[:, None] >= idx[None, :])
        mem = mem0
        outs = []
        for s in range(n_seg):
            xs = x[:, s * seg_len:(s + 1) * seg_len, :].copy()
            h = jnp.concatenate([mem, xs], axis=1)
            q = jnp.einsum('btd,dhe->bhte', h, Wq)
            k = jnp.einsum('btd,dhe->bhte', h, Wk)
            v = jnp.einsum('btd,dhe->bhte', h, Wv)
            scores = jnp.einsum('bhqe,bhke->bhqk', q, k) * scale
            scores = jnp.where(mask[None, None], scores, -1000000000.0)
            p = _softmax(scores, axis=-1)
            o = jnp.einsum('bhqk,bhke->bhqe', p, v)
            o = jnp.einsum('bhte,hed->btd', o, Wo)
            mem = o[:, :M, :].copy()
            outs.append(o[:, M:, :])
        return jnp.concatenate(outs, axis=1)

    def _B_ref(x, w1, w2):
        h = jnp.einsum('bsd,df->bsf', x, w1)
        h = _silu(h)
        out = jnp.einsum('bsf,fd->bsd', h, w2)
        return out
    x = A_x
    xn = _layernorm(x, axis=-1)
    return x + _A_ref(xn, A_mem0, A_Wq, A_Wk, A_Wv, A_Wo, A_seg_len) + _B_ref(xn, B_w1, B_w2)
```

```python
import functools

import jax
import jax.numpy as jnp
from jax import lax
import jax.experimental.pallas as pl
import jax.experimental.pallas.tpu as pltpu

_F32 = jnp.float32
_BF16 = jnp.bfloat16


def _rnd(x):
    return x.astype(_BF16).astype(_F32)


def _kernel(x_ref, mem0_ref, wq_ref, wk_ref, wv_ref, wo_ref, w1_ref, w2_ref,
            o_ref,
            h_scr, q_scr, k_scr, v_scr, att_scr, xn_scr, b_scr,
            *, seg, M, H, Dh, eps):
    L = M + seg
    D = x_ref.shape[-1]
    HD = H * Dh
    i = pl.program_id(1)
    j = pl.program_id(2)

    @pl.when((i == 0) & (j == 0))
    def _init_mem():
        h_scr[0:M, :] = mem0_ref[0].astype(_F32)

    @pl.when(j == 0)
    def _group_init():
        xf = x_ref[...].astype(_F32)
        inv_d = 1.0 / D
        mean = jnp.sum(xf, axis=-1, keepdims=True) * inv_d
        m_b = _rnd(mean)
        cen = xf - mean
        var = jnp.sum(cen * cen, axis=-1, keepdims=True) * inv_d
        v_b = _rnd(var)
        denom = _rnd(jnp.sqrt(_rnd(v_b + _rnd(jnp.float32(eps)))))
        num = _rnd(xf - m_b)
        xn = (num / denom).astype(_BF16)
        xn_scr[...] = xn
        h1 = _rnd(jnp.dot(xn, w1_ref[...], preferred_element_type=_F32))
        sig = _rnd(jax.nn.sigmoid(h1))
        act = (h1 * sig).astype(_BF16)
        b_scr[...] = jnp.dot(act, w2_ref[...], preferred_element_type=_F32).astype(_BF16)

    row0 = pl.multiple_of(j * seg, seg)
    h_scr[M:L, :] = xn_scr[pl.ds(row0, seg), :].astype(_F32)
    hb = h_scr[...].astype(_BF16)
    q_scr[...] = jnp.dot(hb, wq_ref[...], preferred_element_type=_F32).astype(_BF16)
    k_scr[...] = jnp.dot(hb, wk_ref[...], preferred_element_type=_F32).astype(_BF16)
    v_scr[...] = jnp.dot(hb, wv_ref[...], preferred_element_type=_F32).astype(_BF16)

    scale = float(Dh) ** (-0.5)
    row_ids = lax.broadcasted_iota(jnp.int32, (L, L), 0)
    col_ids = lax.broadcasted_iota(jnp.int32, (L, L), 1)
    mask = (row_ids < M) | (row_ids >= col_ids)
    neg = jnp.full((L, L), -1000000000.0, dtype=_F32)

    for hh in range(H):
        q = q_scr[:, hh * Dh:(hh + 1) * Dh]
        k = k_scr[:, hh * Dh:(hh + 1) * Dh]
        v = v_scr[:, hh * Dh:(hh + 1) * Dh]
        s = lax.dot_general(q, k, (((1,), (1,)), ((), ())),
                            preferred_element_type=_F32)
        s = _rnd(s) * scale
        s = jnp.where(mask, s, neg)
        mx = jnp.max(s, axis=-1, keepdims=True)
        p = jnp.exp(s - mx)
        p = p / jnp.sum(p, axis=-1, keepdims=True)
        o = jnp.dot(p.astype(_BF16), v, preferred_element_type=_F32)
        att_scr[:, hh * Dh:(hh + 1) * Dh] = o.astype(_BF16)

    o2 = jnp.dot(att_scr[...], wo_ref[...], preferred_element_type=_F32).astype(_BF16)
    h_scr[0:M, :] = o2[0:M, :].astype(_F32)
    a_out = o2[M:L, :].astype(_F32)
    xr = x_ref[pl.ds(row0, seg), :].astype(_F32)
    br = b_scr[pl.ds(row0, seg), :].astype(_F32)
    out = _rnd(_rnd(xr + a_out) + br)
    o_ref[pl.ds(row0, seg), :] = out.astype(o_ref.dtype)


def pallas_parallel_sum__memory_aug_recurrent_mem_tr__dense_activation_silu__prompt_kernel(
    A_x,
    A_mem0,
    A_Wq,
    A_Wk,
    A_Wv,
    A_Wo,
    A_seg_len,
    B_x,
    B_w1,
    B_w2,
):
    B, S, D = A_x.shape
    H, Dh = A_Wq.shape[1], A_Wq.shape[2]
    M = A_mem0.shape[1]
    seg = int(A_seg_len)
    assert S % seg == 0
    L = M + seg
    n_seg = S // seg
    F = B_w1.shape[1]
    HD = H * Dh

    segs_per_group = 1
    for c in (8, 4, 2):
        if n_seg % c == 0:
            segs_per_group = c
            break
    GROUP = seg * segs_per_group
    n_groups = n_seg // segs_per_group

    x2 = A_x.reshape(B * S, D)
    mem0 = A_mem0.reshape(B, M, D)
    wq = A_Wq.reshape(D, HD)
    wk = A_Wk.reshape(D, HD)
    wv = A_Wv.reshape(D, HD)
    wo = A_Wo.reshape(HD, D)
    w1 = B_w1
    w2 = B_w2

    kernel = functools.partial(_kernel, seg=seg, M=M, H=H, Dh=Dh, eps=1e-05)

    def row_block(b, i, j):
        return (b * n_groups + i, 0)

    def const2(b, i, j):
        return (0, 0)

    def mem_block(b, i, j):
        return (b, 0, 0)

    grid = (B, n_groups, segs_per_group)
    in_specs = [
        pl.BlockSpec((GROUP, D), row_block),
        pl.BlockSpec((1, M, D), mem_block),
        pl.BlockSpec((D, HD), const2),
        pl.BlockSpec((D, HD), const2),
        pl.BlockSpec((D, HD), const2),
        pl.BlockSpec((HD, D), const2),
        pl.BlockSpec((D, F), const2),
        pl.BlockSpec((F, D), const2),
    ]
    out_specs = pl.BlockSpec((GROUP, D), row_block)
    scratch_shapes = [
        pltpu.VMEM((L, D), _F32),
        pltpu.VMEM((L, HD), _BF16),
        pltpu.VMEM((L, HD), _BF16),
        pltpu.VMEM((L, HD), _BF16),
        pltpu.VMEM((L, HD), _BF16),
        pltpu.VMEM((GROUP, D), _BF16),
        pltpu.VMEM((GROUP, D), _BF16),
    ]

    out = pl.pallas_call(
        kernel,
        grid=grid,
        in_specs=in_specs,
        out_specs=out_specs,
        out_shape=jax.ShapeDtypeStruct((B * S, D), A_x.dtype),
        scratch_shapes=scratch_shapes,
        compiler_params=pltpu.CompilerParams(
            dimension_semantics=("arbitrary", "arbitrary", "arbitrary"),
            vmem_limit_bytes=100 * 1024 * 1024,
        ),
    )(x2, mem0, wq, wk, wv, wo, w1, w2)
    return out.reshape(B, S, D)
```

```python
import contextlib
import functools

import jax
import jax.numpy as jnp
from jax import lax
import jax.experimental.pallas as pl
import jax.experimental.pallas.tpu as pltpu

_F32 = jnp.float32
_BF16 = jnp.bfloat16


def _rnd(x):
    return x.astype(_BF16).astype(_F32)


def _kernel(x_ref, mem0_ref, wq_ref, wk_ref, wv_ref, wo_ref, w1_ref, w2T_ref,
            o_ref,
            lhs_scr, q_buf, k_buf, v_buf, att_scr, xn_scr, b_scr,
            *, seg, M, H, Dh, eps, fwd, wf, scopes=False):
    def scope(name):
        return jax.named_scope(name) if scopes else contextlib.nullcontext()

    L = M + seg
    D = x_ref.shape[-1]
    i = pl.program_id(1)
    j = pl.program_id(2)
    par = lax.rem(j, 2)

    @pl.when((i == 0) & (j == 0))
    def _init_mem():
        lhs_scr[0:M, :] = mem0_ref[0].astype(_F32)

    @pl.when(j == 0)
    def _group_init():
        with scope("group_init"):
            xf = x_ref[...].astype(_F32)
            inv_d = 1.0 / D
            mean = jnp.sum(xf, axis=-1, keepdims=True) * inv_d
            m_b = _rnd(mean)
            cen = xf - mean
            var = jnp.sum(cen * cen, axis=-1, keepdims=True) * inv_d
            v_b = _rnd(var)
            denom = _rnd(jnp.sqrt(_rnd(v_b + _rnd(jnp.float32(eps)))))
            num = _rnd(xf - m_b)
            xn = _rnd(num / denom)
            xn_scr[...] = xn
            xnb = xn.astype(_BF16)
            h1 = _rnd(jnp.dot(xnb, w1_ref[...], preferred_element_type=_F32))
            sig = _rnd(jax.nn.sigmoid(h1))
            act = (h1 * sig).astype(_BF16)
            b_scr[...] = lax.dot_general(
                act, w2T_ref[...], (((1,), (1,)), ((), ())),
                preferred_element_type=_F32).astype(_BF16)

    row0 = pl.multiple_of(j * seg, seg)

    def _project(nx, start):
        lhs_scr[M:M + nx, :] = xn_scr[pl.ds(pl.multiple_of(start, 8), nx), :]
        hb = lhs_scr[0:M + nx, :].astype(_BF16)
        rq = jnp.dot(hb, wq_ref[...], preferred_element_type=_F32).astype(_BF16)
        rk = jnp.dot(hb, wk_ref[...], preferred_element_type=_F32).astype(_BF16)
        rv = jnp.dot(hb, wv_ref[...], preferred_element_type=_F32).astype(_BF16)
        return rq, rk, rv

    with scope("qkv_proj"):
        if fwd > 0:
            @pl.when(par == 0)
            def _even():
                nx = seg + fwd
                rq, rk, rv = _project(nx, row0)
                q_buf[0, 0:L, :] = rq[0:L]
                k_buf[0, 0:L, :] = rk[0:L]
                v_buf[0, 0:L, :] = rv[0:L]
                q_buf[1, M:M + fwd, :] = rq[L:L + fwd]
                k_buf[1, M:M + fwd, :] = rk[L:L + fwd]
                v_buf[1, M:M + fwd, :] = rv[L:L + fwd]

            @pl.when(par == 1)
            def _odd():
                nx = seg - fwd
                rq, rk, rv = _project(nx, row0 + fwd)
                q_buf[1, 0:M, :] = rq[0:M]
                k_buf[1, 0:M, :] = rk[0:M]
                v_buf[1, 0:M, :] = rv[0:M]
                q_buf[1, M + fwd:L, :] = rq[M:M + nx]
                k_buf[1, M + fwd:L, :] = rk[M:M + nx]
                v_buf[1, M + fwd:L, :] = rv[M:M + nx]
        else:
            rq, rk, rv = _project(seg, row0)
            q_buf[0, :, :] = rq
            k_buf[0, :, :] = rk
            v_buf[0, :, :] = rv

    bufi = par if fwd > 0 else 0

    scale = float(Dh) ** (-0.5)
    row_ids = lax.broadcasted_iota(jnp.int32, (L, L), 0)
    col_ids = lax.broadcasted_iota(jnp.int32, (L, L), 1)
    mask = (row_ids < M) | (row_ids >= col_ids)
    neg = jnp.full((L, L), -1000000000.0, dtype=_F32)

    def _scores(hh):
        q = q_buf[bufi, :, hh * Dh:(hh + 1) * Dh]
        k = k_buf[bufi, :, hh * Dh:(hh + 1) * Dh]
        return lax.dot_general(q, k, (((1,), (1,)), ((), ())),
                               preferred_element_type=_F32)

    def _finish(hh, s):
        v = v_buf[bufi, :, hh * Dh:(hh + 1) * Dh]
        s = jnp.where(mask, s, neg)
        mx = jnp.max(s, axis=-1, keepdims=True)
        pb = jnp.exp((s - mx) * scale).astype(_BF16)
        ou = jnp.dot(pb, v, preferred_element_type=_F32)
        denom = jnp.sum(pb.astype(_F32), axis=-1, keepdims=True)
        att_scr[0:L, hh * Dh:(hh + 1) * Dh] = (ou / denom).astype(_BF16)

    with scope("attention"):
        s_next = _scores(0)
        for hh in range(H):
            s_cur = s_next
            if hh + 1 < H:
                s_next = _scores(hh + 1)
            _finish(hh, s_cur)

    def _emit(lhs_rows):
        o2 = jnp.dot(lhs_rows, wo_ref[...], preferred_element_type=_F32).astype(_BF16)
        lhs_scr[0:M, :] = o2[0:M, :].astype(_F32)
        return o2[M:, :].astype(_F32)

    def _residual(start, a_out):
        n = a_out.shape[0]
        xr = x_ref[pl.ds(start, n), :].astype(_F32)
        br = b_scr[pl.ds(start, n), :].astype(_F32)
        out = _rnd(_rnd(xr + a_out) + br)
        o_ref[pl.ds(start, n), :] = out.astype(o_ref.dtype)

    with scope("wo_out"):
        if wf > 0:
            @pl.when(par == 0)
            def _out_even():
                a_out = _emit(att_scr[0:L - wf, :])
                _residual(row0, a_out)
                att_scr[L:L + wf, :] = att_scr[L - wf:L, :]

            @pl.when(par == 1)
            def _out_odd():
                a_out = _emit(att_scr[0:L + wf, :])
                _residual(row0, a_out[0:seg])
                _residual(row0 - wf, a_out[seg:])
        else:
            a_out = _emit(att_scr[0:L, :])
            _residual(row0, a_out)


def pallas_parallel_sum__memory_aug_recurrent_mem_tr__dense_activation_silu__prompt_kernel(
    A_x,
    A_mem0,
    A_Wq,
    A_Wk,
    A_Wv,
    A_Wo,
    A_seg_len,
    B_x,
    B_w1,
    B_w2,
    _scopes=False,
):
    B, S, D = A_x.shape
    H, Dh = A_Wq.shape[1], A_Wq.shape[2]
    M = A_mem0.shape[1]
    seg = int(A_seg_len)
    assert S % seg == 0
    L = M + seg
    n_seg = S // seg
    F = B_w1.shape[1]
    HD = H * Dh

    segs_per_group = 1
    for c in (16, 8, 4, 2):
        if n_seg % c == 0:
            segs_per_group = c
            break
    GROUP = seg * segs_per_group
    n_groups = n_seg // segs_per_group

    fwd = (-L) % 16
    if not (segs_per_group % 2 == 0 and 0 < fwd < seg and fwd % 8 == 0 and M % 8 == 0
            and (seg - fwd) % 8 == 0):
        fwd = 0
    nbuf = 2 if fwd > 0 else 1
    wf = fwd

    x2 = A_x.reshape(B * S, D)
    mem0 = A_mem0.reshape(B, M, D)
    wq = A_Wq.reshape(D, HD)
    wk = A_Wk.reshape(D, HD)
    wv = A_Wv.reshape(D, HD)
    wo = A_Wo.reshape(HD, D)
    w1 = B_w1
    w2T = jnp.swapaxes(B_w2, 0, 1)

    kernel = functools.partial(_kernel, seg=seg, M=M, H=H, Dh=Dh, eps=1e-05,
                               fwd=fwd, wf=wf, scopes=_scopes)

    def row_block(b, i, j):
        return (b * n_groups + i, 0)

    def const2(b, i, j):
        return (0, 0)

    def mem_block(b, i, j):
        return (b, 0, 0)

    grid = (B, n_groups, segs_per_group)
    in_specs = [
        pl.BlockSpec((GROUP, D), row_block),
        pl.BlockSpec((1, M, D), mem_block),
        pl.BlockSpec((D, HD), const2),
        pl.BlockSpec((D, HD), const2),
        pl.BlockSpec((D, HD), const2),
        pl.BlockSpec((HD, D), const2),
        pl.BlockSpec((D, F), const2),
        pl.BlockSpec((D, F), const2),
    ]
    out_specs = pl.BlockSpec((GROUP, D), row_block)
    scratch_shapes = [
        pltpu.VMEM((L + fwd, D), _F32),
        pltpu.VMEM((nbuf, L, HD), _BF16),
        pltpu.VMEM((nbuf, L, HD), _BF16),
        pltpu.VMEM((nbuf, L, HD), _BF16),
        pltpu.VMEM((L + wf, HD), _BF16),
        pltpu.VMEM((GROUP, D), _F32),
        pltpu.VMEM((GROUP, D), _BF16),
    ]

    out = pl.pallas_call(
        kernel,
        grid=grid,
        in_specs=in_specs,
        out_specs=out_specs,
        out_shape=jax.ShapeDtypeStruct((B * S, D), A_x.dtype),
        scratch_shapes=scratch_shapes,
        compiler_params=pltpu.CompilerParams(
            dimension_semantics=("arbitrary", "arbitrary", "arbitrary"),
            vmem_limit_bytes=100 * 1024 * 1024,
        ),
    )(x2, mem0, wq, wk, wv, wo, w1, w2T)
    return out.reshape(B, S, D)
```

```python
import contextlib
import functools

import jax
import jax.numpy as jnp
from jax import lax
import jax.experimental.pallas as pl
import jax.experimental.pallas.tpu as pltpu

_F32 = jnp.float32
_BF16 = jnp.bfloat16
LOOKAHEAD = 2


def _rnd(x):
    return x.astype(_BF16).astype(_F32)


def _kernel(x_ref, mem0_ref, wq_ref, wk_ref, wv_ref, wo_ref, w1_ref, w2T_ref,
            o_ref,
            lhs_scr, q_buf, k_buf, v_buf, att_scr, xn_scr, b_scr,
            *, seg, M, H, Dh, eps, fwd, wf, scopes=False):
    def scope(name):
        return jax.named_scope(name) if scopes else contextlib.nullcontext()

    L = M + seg
    D = x_ref.shape[-1]
    i = pl.program_id(1)
    j = pl.program_id(2)
    par = lax.rem(j, 2)

    @pl.when((i == 0) & (j == 0))
    def _init_mem():
        lhs_scr[0:M, :] = mem0_ref[0].astype(_F32)

    @pl.when(j == 0)
    def _group_init():
        with scope("group_init"):
            xf = x_ref[...].astype(_F32)
            inv_d = 1.0 / D
            mean = jnp.sum(xf, axis=-1, keepdims=True) * inv_d
            m_b = _rnd(mean)
            cen = xf - mean
            var = jnp.sum(cen * cen, axis=-1, keepdims=True) * inv_d
            v_b = _rnd(var)
            denom = _rnd(jnp.sqrt(_rnd(v_b + _rnd(jnp.float32(eps)))))
            num = _rnd(xf - m_b)
            xn = _rnd(num / denom)
            xn_scr[...] = xn
            xnb = xn.astype(_BF16)
            h1 = _rnd(jnp.dot(xnb, w1_ref[...], preferred_element_type=_F32))
            sig = _rnd(jax.nn.sigmoid(h1))
            act = (h1 * sig).astype(_BF16)
            b_scr[...] = lax.dot_general(
                act, w2T_ref[...], (((1,), (1,)), ((), ())),
                preferred_element_type=_F32).astype(_BF16)

    row0 = pl.multiple_of(j * seg, seg)

    def _project(nx, start):
        lhs_scr[M:M + nx, :] = xn_scr[pl.ds(pl.multiple_of(start, 8), nx), :]
        hb = lhs_scr[0:M + nx, :].astype(_BF16)
        rq = jnp.dot(hb, wq_ref[...], preferred_element_type=_F32).astype(_BF16)
        rk = jnp.dot(hb, wk_ref[...], preferred_element_type=_F32).astype(_BF16)
        rv = jnp.dot(hb, wv_ref[...], preferred_element_type=_F32).astype(_BF16)
        return rq, rk, rv

    with scope("qkv_proj"):
        if fwd > 0:
            @pl.when(par == 0)
            def _even():
                nx = seg + fwd
                rq, rk, rv = _project(nx, row0)
                q_buf[0, 0:L, :] = rq[0:L]
                k_buf[0, 0:L, :] = rk[0:L]
                v_buf[0, 0:L, :] = rv[0:L]
                q_buf[1, M:M + fwd, :] = rq[L:L + fwd]
                k_buf[1, M:M + fwd, :] = rk[L:L + fwd]
                v_buf[1, M:M + fwd, :] = rv[L:L + fwd]

            @pl.when(par == 1)
            def _odd():
                nx = seg - fwd
                rq, rk, rv = _project(nx, row0 + fwd)
                q_buf[1, 0:M, :] = rq[0:M]
                k_buf[1, 0:M, :] = rk[0:M]
                v_buf[1, 0:M, :] = rv[0:M]
                q_buf[1, M + fwd:L, :] = rq[M:M + nx]
                k_buf[1, M + fwd:L, :] = rk[M:M + nx]
                v_buf[1, M + fwd:L, :] = rv[M:M + nx]
        else:
            rq, rk, rv = _project(seg, row0)
            q_buf[0, :, :] = rq
            k_buf[0, :, :] = rk
            v_buf[0, :, :] = rv

    bufi = par if fwd > 0 else 0

    scale = float(Dh) ** (-0.5)
    row_ids = lax.broadcasted_iota(jnp.int32, (L, L), 0)
    col_ids = lax.broadcasted_iota(jnp.int32, (L, L), 1)
    mask = (row_ids < M) | (row_ids >= col_ids)
    neg = jnp.full((L, L), -1000000000.0, dtype=_F32)

    def _scores(hh):
        q = q_buf[bufi, :, hh * Dh:(hh + 1) * Dh]
        k = k_buf[bufi, :, hh * Dh:(hh + 1) * Dh]
        return lax.dot_general(q, k, (((1,), (1,)), ((), ())),
                               preferred_element_type=_F32)

    def _finish(hh, s):
        v = v_buf[bufi, :, hh * Dh:(hh + 1) * Dh]
        s = jnp.where(mask, s, neg)
        mx = jnp.max(s, axis=-1, keepdims=True)
        pb = jnp.exp((s - mx) * scale).astype(_BF16)
        ou = jnp.dot(pb, v, preferred_element_type=_F32)
        denom = jnp.sum(pb.astype(_F32), axis=-1, keepdims=True)
        att_scr[0:L, hh * Dh:(hh + 1) * Dh] = (ou / denom).astype(_BF16)

    with scope("attention"):
        pending = [_scores(hh) for hh in range(min(LOOKAHEAD, H))]
        for hh in range(H):
            s_cur = pending.pop(0)
            if hh + LOOKAHEAD < H:
                pending.append(_scores(hh + LOOKAHEAD))
            _finish(hh, s_cur)

    def _emit(lhs_rows):
        o2 = jnp.dot(lhs_rows, wo_ref[...], preferred_element_type=_F32).astype(_BF16)
        lhs_scr[0:M, :] = o2[0:M, :].astype(_F32)
        return o2[M:, :].astype(_F32)

    def _residual(start, a_out):
        n = a_out.shape[0]
        xr = x_ref[pl.ds(start, n), :].astype(_F32)
        br = b_scr[pl.ds(start, n), :].astype(_F32)
        out = _rnd(_rnd(xr + a_out) + br)
        o_ref[pl.ds(start, n), :] = out.astype(o_ref.dtype)

    with scope("wo_out"):
        if wf > 0:
            @pl.when(par == 0)
            def _out_even():
                a_out = _emit(att_scr[0:L - wf, :])
                _residual(row0, a_out)
                att_scr[L:L + wf, :] = att_scr[L - wf:L, :]

            @pl.when(par == 1)
            def _out_odd():
                a_out = _emit(att_scr[0:L + wf, :])
                _residual(row0, a_out[0:seg])
                _residual(row0 - wf, a_out[seg:])
        else:
            a_out = _emit(att_scr[0:L, :])
            _residual(row0, a_out)


def pallas_parallel_sum__memory_aug_recurrent_mem_tr__dense_activation_silu__prompt_kernel(
    A_x,
    A_mem0,
    A_Wq,
    A_Wk,
    A_Wv,
    A_Wo,
    A_seg_len,
    B_x,
    B_w1,
    B_w2,
    _scopes=False,
):
    B, S, D = A_x.shape
    H, Dh = A_Wq.shape[1], A_Wq.shape[2]
    M = A_mem0.shape[1]
    seg = int(A_seg_len)
    assert S % seg == 0
    L = M + seg
    n_seg = S // seg
    F = B_w1.shape[1]
    HD = H * Dh

    segs_per_group = 1
    for c in (16, 8, 4, 2):
        if n_seg % c == 0:
            segs_per_group = c
            break
    GROUP = seg * segs_per_group
    n_groups = n_seg // segs_per_group

    fwd = (-L) % 16
    if not (segs_per_group % 2 == 0 and 0 < fwd < seg and fwd % 8 == 0 and M % 8 == 0
            and (seg - fwd) % 8 == 0):
        fwd = 0
    nbuf = 2 if fwd > 0 else 1
    wf = fwd

    x2 = A_x.reshape(B * S, D)
    mem0 = A_mem0.reshape(B, M, D)
    wq = A_Wq.reshape(D, HD)
    wk = A_Wk.reshape(D, HD)
    wv = A_Wv.reshape(D, HD)
    wo = A_Wo.reshape(HD, D)
    w1 = B_w1
    w2T = jnp.swapaxes(B_w2, 0, 1)

    kernel = functools.partial(_kernel, seg=seg, M=M, H=H, Dh=Dh, eps=1e-05,
                               fwd=fwd, wf=wf, scopes=_scopes)

    def row_block(b, i, j):
        return (b * n_groups + i, 0)

    def const2(b, i, j):
        return (0, 0)

    def mem_block(b, i, j):
        return (b, 0, 0)

    grid = (B, n_groups, segs_per_group)
    in_specs = [
        pl.BlockSpec((GROUP, D), row_block),
        pl.BlockSpec((1, M, D), mem_block),
        pl.BlockSpec((D, HD), const2),
        pl.BlockSpec((D, HD), const2),
        pl.BlockSpec((D, HD), const2),
        pl.BlockSpec((HD, D), const2),
        pl.BlockSpec((D, F), const2),
        pl.BlockSpec((D, F), const2),
    ]
    out_specs = pl.BlockSpec((GROUP, D), row_block)
    scratch_shapes = [
        pltpu.VMEM((L + fwd, D), _F32),
        pltpu.VMEM((nbuf, L, HD), _BF16),
        pltpu.VMEM((nbuf, L, HD), _BF16),
        pltpu.VMEM((nbuf, L, HD), _BF16),
        pltpu.VMEM((L + wf, HD), _BF16),
        pltpu.VMEM((GROUP, D), _F32),
        pltpu.VMEM((GROUP, D), _BF16),
    ]

    out = pl.pallas_call(
        kernel,
        grid=grid,
        in_specs=in_specs,
        out_specs=out_specs,
        out_shape=jax.ShapeDtypeStruct((B * S, D), A_x.dtype),
        scratch_shapes=scratch_shapes,
        compiler_params=pltpu.CompilerParams(
            dimension_semantics=("arbitrary", "arbitrary", "arbitrary"),
            vmem_limit_bytes=100 * 1024 * 1024,
        ),
    )(x2, mem0, wq, wk, wv, wo, w1, w2T)
    return out.reshape(B, S, D)
```

```python
import functools

import jax
import jax.numpy as jnp
from jax import lax
import jax.experimental.pallas as pl
import jax.experimental.pallas.tpu as pltpu

_F32 = jnp.float32
_BF16 = jnp.bfloat16
LOOKAHEAD = 2


def _rnd(x):
    return x.astype(_BF16).astype(_F32)


def _kernel(x_ref, mem0_ref, wq_ref, wk_ref, wv_ref, wo_ref, w1_ref, w2T_ref,
            o_ref,
            lhs_scr, q_buf, k_buf, v_buf, att_scr, xn_scr, b_scr,
            *, seg, M, H, Dh, eps, fwd, wf):
    L = M + seg
    D = x_ref.shape[-1]
    i = pl.program_id(1)
    j = pl.program_id(2)
    par = lax.rem(j, 2)

    @pl.when((i == 0) & (j == 0))
    def _init_mem():
        lhs_scr[0:M, :] = mem0_ref[0].astype(_F32)

    @pl.when(j == 0)
    def _group_init():
        xf = x_ref[...].astype(_F32)
        inv_d = 1.0 / D
        mean = jnp.sum(xf, axis=-1, keepdims=True) * inv_d
        m_b = _rnd(mean)
        cen = xf - mean
        var = jnp.sum(cen * cen, axis=-1, keepdims=True) * inv_d
        v_b = _rnd(var)
        denom = _rnd(jnp.sqrt(_rnd(v_b + _rnd(jnp.float32(eps)))))
        num = _rnd(xf - m_b)
        xn = _rnd(num / denom)
        xn_scr[...] = xn
        xnb = xn.astype(_BF16)
        h1 = _rnd(jnp.dot(xnb, w1_ref[...], preferred_element_type=_F32))
        sig = _rnd(jax.nn.sigmoid(h1))
        act = (h1 * sig).astype(_BF16)
        b_scr[...] = lax.dot_general(
            act, w2T_ref[...], (((1,), (1,)), ((), ())),
            preferred_element_type=_F32).astype(_BF16)

    row0 = pl.multiple_of(j * seg, seg)

    def _project(nx, start):
        lhs_scr[M:M + nx, :] = xn_scr[pl.ds(pl.multiple_of(start, 8), nx), :]
        hb = lhs_scr[0:M + nx, :].astype(_BF16)
        rq = jnp.dot(hb, wq_ref[...], preferred_element_type=_F32).astype(_BF16)
        rk = jnp.dot(hb, wk_ref[...], preferred_element_type=_F32).astype(_BF16)
        rv = jnp.dot(hb, wv_ref[...], preferred_element_type=_F32).astype(_BF16)
        return rq, rk, rv

    if fwd > 0:
        @pl.when(par == 0)
        def _even():
            nx = seg + fwd
            rq, rk, rv = _project(nx, row0)
            q_buf[0, 0:L, :] = rq[0:L]
            k_buf[0, 0:L, :] = rk[0:L]
            v_buf[0, 0:L, :] = rv[0:L]
            q_buf[1, M:M + fwd, :] = rq[L:L + fwd]
            k_buf[1, M:M + fwd, :] = rk[L:L + fwd]
            v_buf[1, M:M + fwd, :] = rv[L:L + fwd]

        @pl.when(par == 1)
        def _odd():
            nx = seg - fwd
            rq, rk, rv = _project(nx, row0 + fwd)
            q_buf[1, 0:M, :] = rq[0:M]
            k_buf[1, 0:M, :] = rk[0:M]
            v_buf[1, 0:M, :] = rv[0:M]
            q_buf[1, M + fwd:L, :] = rq[M:M + nx]
            k_buf[1, M + fwd:L, :] = rk[M:M + nx]
            v_buf[1, M + fwd:L, :] = rv[M:M + nx]
    else:
        rq, rk, rv = _project(seg, row0)
        q_buf[0, :, :] = rq
        k_buf[0, :, :] = rk
        v_buf[0, :, :] = rv

    bufi = par if fwd > 0 else 0

    scale = float(Dh) ** (-0.5)
    row_ids = lax.broadcasted_iota(jnp.int32, (L, L), 0)
    col_ids = lax.broadcasted_iota(jnp.int32, (L, L), 1)
    mask = (row_ids < M) | (row_ids >= col_ids)
    neg = jnp.full((L, L), -1000000000.0, dtype=_F32)

    def _scores(hh):
        q = q_buf[bufi, :, hh * Dh:(hh + 1) * Dh]
        k = k_buf[bufi, :, hh * Dh:(hh + 1) * Dh]
        return lax.dot_general(q, k, (((1,), (1,)), ((), ())),
                               preferred_element_type=_F32)

    def _finish(hh, s):
        v = v_buf[bufi, :, hh * Dh:(hh + 1) * Dh]
        s = jnp.where(mask, s, neg)
        mx = jnp.max(s, axis=-1, keepdims=True)
        pb = jnp.exp((s - mx) * scale).astype(_BF16)
        ou = jnp.dot(pb, v, preferred_element_type=_F32)
        denom = jnp.sum(pb.astype(_F32), axis=-1, keepdims=True)
        att_scr[0:L, hh * Dh:(hh + 1) * Dh] = (ou / denom).astype(_BF16)

    pending = [_scores(hh) for hh in range(min(LOOKAHEAD, H))]
    for hh in range(H):
        s_cur = pending.pop(0)
        if hh + LOOKAHEAD < H:
            pending.append(_scores(hh + LOOKAHEAD))
        _finish(hh, s_cur)

    def _emit(lhs_rows):
        o2 = jnp.dot(lhs_rows, wo_ref[...], preferred_element_type=_F32).astype(_BF16)
        lhs_scr[0:M, :] = o2[0:M, :].astype(_F32)
        return o2[M:, :].astype(_F32)

    def _residual(start, a_out):
        n = a_out.shape[0]
        xr = x_ref[pl.ds(start, n), :].astype(_F32)
        br = b_scr[pl.ds(start, n), :].astype(_F32)
        out = _rnd(_rnd(xr + a_out) + br)
        o_ref[pl.ds(start, n), :] = out.astype(o_ref.dtype)

    if wf > 0:
        @pl.when(par == 0)
        def _out_even():
            a_out = _emit(att_scr[0:L - wf, :])
            _residual(row0, a_out)
            att_scr[L:L + wf, :] = att_scr[L - wf:L, :]

        @pl.when(par == 1)
        def _out_odd():
            a_out = _emit(att_scr[0:L + wf, :])
            _residual(row0, a_out[0:seg])
            _residual(row0 - wf, a_out[seg:])
    else:
        a_out = _emit(att_scr[0:L, :])
        _residual(row0, a_out)


def pallas_parallel_sum__memory_aug_recurrent_mem_tr__dense_activation_silu__prompt_kernel(
    A_x,
    A_mem0,
    A_Wq,
    A_Wk,
    A_Wv,
    A_Wo,
    A_seg_len,
    B_x,
    B_w1,
    B_w2,
):
    B, S, D = A_x.shape
    H, Dh = A_Wq.shape[1], A_Wq.shape[2]
    M = A_mem0.shape[1]
    seg = int(A_seg_len)
    assert S % seg == 0
    L = M + seg
    n_seg = S // seg
    F = B_w1.shape[1]
    HD = H * Dh

    segs_per_group = 1
    for c in (16, 8, 4, 2):
        if n_seg % c == 0:
            segs_per_group = c
            break
    GROUP = seg * segs_per_group
    n_groups = n_seg // segs_per_group

    fwd = (-L) % 16
    if not (segs_per_group % 2 == 0 and 0 < fwd < seg and fwd % 8 == 0 and M % 8 == 0
            and (seg - fwd) % 8 == 0):
        fwd = 0
    nbuf = 2 if fwd > 0 else 1
    wf = fwd

    x2 = A_x.reshape(B * S, D)
    mem0 = A_mem0.reshape(B, M, D)
    wq = A_Wq.reshape(D, HD)
    wk = A_Wk.reshape(D, HD)
    wv = A_Wv.reshape(D, HD)
    wo = A_Wo.reshape(HD, D)
    w1 = B_w1
    w2T = jnp.swapaxes(B_w2, 0, 1)

    kernel = functools.partial(_kernel, seg=seg, M=M, H=H, Dh=Dh, eps=1e-05,
                               fwd=fwd, wf=wf)

    def row_block(b, i, j):
        return (b * n_groups + i, 0)

    def const2(b, i, j):
        return (0, 0)

    def mem_block(b, i, j):
        return (b, 0, 0)

    grid = (B, n_groups, segs_per_group)
    in_specs = [
        pl.BlockSpec((GROUP, D), row_block),
        pl.BlockSpec((1, M, D), mem_block),
        pl.BlockSpec((D, HD), const2),
        pl.BlockSpec((D, HD), const2),
        pl.BlockSpec((D, HD), const2),
        pl.BlockSpec((HD, D), const2),
        pl.BlockSpec((D, F), const2),
        pl.BlockSpec((D, F), const2),
    ]
    out_specs = pl.BlockSpec((GROUP, D), row_block)
    scratch_shapes = [
        pltpu.VMEM((L + fwd, D), _F32),
        pltpu.VMEM((nbuf, L, HD), _BF16),
        pltpu.VMEM((nbuf, L, HD), _BF16),
        pltpu.VMEM((nbuf, L, HD), _BF16),
        pltpu.VMEM((L + wf, HD), _BF16),
        pltpu.VMEM((GROUP, D), _F32),
        pltpu.VMEM((GROUP, D), _BF16),
    ]

    out = pl.pallas_call(
        kernel,
        grid=grid,
        in_specs=in_specs,
        out_specs=out_specs,
        out_shape=jax.ShapeDtypeStruct((B * S, D), A_x.dtype),
        scratch_shapes=scratch_shapes,
        compiler_params=pltpu.CompilerParams(
            dimension_semantics=("arbitrary", "arbitrary", "arbitrary"),
            vmem_limit_bytes=100 * 1024 * 1024,
        ),
    )(x2, mem0, wq, wk, wv, wo, w1, w2T)
    return out.reshape(B, S, D)
```
